```python
import os as _os
_os.environ.setdefault('JAX_PLATFORMS', 'cpu')
import jax
import jax.numpy as jnp

def _softmax(x, axis=-1):
    return jax.nn.softmax(x, axis=axis)

def _gelu(x):
    return jax.nn.gelu(x, approximate=True)

def _silu(x):
    return jax.nn.silu(x)

def _sigmoid(x):
    return jax.nn.sigmoid(x)

def _layernorm(x, axis=-1, eps=1e-05):
    m = jnp.mean(x, axis=axis, keepdims=True)
    v = jnp.var(x, axis=axis, keepdims=True)
    return (x - m) / jnp.sqrt(v + eps)

def _scatter_add(tgt, idx, src, axis=0):
    return tgt.at[idx].add(src)

def _segment_sum(src, seg, n):
    return jax.ops.segment_sum(src, seg, n)

class _Rng:

    def __init__(self, key):
        self._k = key

    def _next(self):
        self._k, sub = jax.random.split(self._k)
        return sub

    def normal(self, shape):
        return jax.random.normal(self._next(), shape, dtype=jnp.bfloat16)

    def randint(self, lo, hi, shape):
        return jax.random.randint(self._next(), shape, lo, hi, dtype=jnp.int32)

    def uniform(self, shape, lo=0.0, hi=1.0):
        return jax.random.uniform(self._next(), shape, jnp.bfloat16, lo, hi)

    def permutation(self, n):
        return jax.random.permutation(self._next(), n)
kernel_name = 'adaLN_cond__linear_attn_block__swiglu_ffn__prompt'

def setup_inputs():
    _rng = _Rng(jax.random.key(int.from_bytes(__import__("os").urandom(4), "little")))
    _w = lambda a: (lambda t: t.astype(jnp.bfloat16) if jnp.issubdtype(t.dtype, jnp.floating) else t)(jnp.asarray(a))

    def _A_setup():
        B, S, D = (1, 2048, 640)
        return {'x': _w((lambda *s: _rng.normal(s) * 0.05)(B, S, D)), 'wqkv': _w((lambda *s: _rng.normal(s) * 0.8)(D, 3 * D)), 'wo': _w((lambda *s: _rng.normal(s) * 0.05)(D, D))}
    _A_in = _A_setup()

    def _B_setup():
        B, S, D, F = (1, 2048, 640, 1728)
        return {'x': _w((lambda *s: _rng.normal(s) * 0.05)(B, S, D)), 'w_gate': _w((lambda *s: _rng.normal(s) * 0.05)(D, F)), 'w_up': _w((lambda *s: _rng.normal(s) * 0.05)(D, F)), 'w_down': _w((lambda *s: _rng.normal(s) * 0.05)(F, D))}
    _B_in = _B_setup()
    return {'A_x': _A_in['x'], 'A_wqkv': _A_in['wqkv'], 'A_wo': _A_in['wo'], 'B_x': _B_in['x'], 'B_w_gate': _B_in['w_gate'], 'B_w_up': _B_in['w_up'], 'B_w_down': _B_in['w_down'], 'c': _w((lambda *s: _rng.normal(s) * 0.05)(1, 640) * 8.0), 'w_mod': _w((lambda *s: _rng.normal(s) * 0.05)(640, 6 * 640) * 640 ** (-0.5) * 8.0)}

def reference(A_x, A_wqkv, A_wo, B_x, B_w_gate, B_w_up, B_w_down, c, w_mod):

    def _A_ref(x, wqkv, wo):
        B, S, D = x.shape
        H = 32
        Dh = D // H
        qkv = (lambda x, *d: x.transpose(*d))((x @ wqkv).reshape(B, S, 3, H, Dh), 2, 0, 3, 1, 4)
        q, k, v = (qkv[0], qkv[1], qkv[2])
        phi = lambda t: jnp.where(t > 0, t + 1, jnp.exp(t)) + 1e-06
        pq, pk = (phi(q), phi(k))
        kv = jnp.einsum('bhsd,bhse->bhde', pk, v)
        z = jnp.einsum('bhsd->bhd', pk)
        num = jnp.einsum('bhqd,bhde->bhqe', pq, kv)
        den = jnp.einsum('bhqd,bhd->bhq', pq, z)[..., None] + 1e-06
        o = num / den
        return (lambda x, *d: x.transpose(*d))(o, 0, 2, 1, 3).reshape(B, S, D) @ wo

    def _B_ref(x, w_gate, w_up, w_down):
        g = _silu(x @ w_gate)
        u = x @ w_up
        return g * u @ w_down
    x = A_x
    mod = (_silu(c) @ w_mod).reshape(c.shape[0], 6, 1, -1)
    sa, ca, ga, sb, cb, gb = (mod[:, 0].copy(), mod[:, 1].copy(), mod[:, 2].copy(), mod[:, 3].copy(), mod[:, 4].copy(), mod[:, 5].copy())
    h = _layernorm(x, axis=-1) * (1 + ca) + sa
    x = x + ga * _A_ref(h, A_wqkv, A_wo)
    h = _layernorm(x, axis=-1) * (1 + cb) + sb
    x = x + gb * _B_ref(h, B_w_gate, B_w_up, B_w_down)
    return x
```

```python
import jax
import jax.numpy as jnp
import jax.experimental.pallas as pl
import jax.experimental.pallas.tpu as pltpu

F32, BF16 = jnp.float32, jnp.bfloat16
S, D, F, DH = 2048, 640, 1728, 20
L = 128
TM = 4 * L
NT = S // TM
RB = D // 4
GU_CHUNKS = [(256 * q, 128) for q in range(6)] + [(1536, 96)]
pieces = lambda rows, most: [(r0, min(most, rows - r0)) for r0 in range(0, rows, most)]
P_PIECES, G_PIECES, D_PIECES = pieces(RB, 64), pieces(RB, 80), pieces(RB // 2, 48)


D_GROUPS = [(0, 3), (6, 2), (10, 2)]


def feature(split, i, r, blocks=4):
    r0, rows = [p for p in split if p[0] <= r][-1]
    return blocks * r0 + i * rows + r - r0


HEAD_ROWS = [(0, 144), (112, 272), (240, 400), (368, 528), (496, 640)]


def s_a(a11, a12, a21, a22, only):
    return (lambda: a11 + a22, lambda: a21 + a22, lambda: a11, lambda: a22,
            lambda: a11 + a12, lambda: a21 - a11, lambda: a12 - a22)[only]()


def s_b(b11, b12, b21, b22, only):
    return (lambda: b11 + b22, lambda: b11, lambda: b12 - b22, lambda: b21 - b11,
            lambda: b22, lambda: b11 + b12, lambda: b21 + b22)[only]()


def s_ct(c11, c12, c21, c22, only):
    return (lambda: c11 + c22, lambda: c21 - c22, lambda: c12 + c22, lambda: c11 + c21,
            lambda: c12 - c11, lambda: c22, lambda: c11)[only]()


S_A = (s_a, [(2, [0]), (3, [3]), (0, []), (1, [2]), (5, []), (4, [1]), (6, [])])
S_B = (s_b, [(1, [0]), (4, [3]), (0, []), (2, [1]), (5, []), (3, [2]), (6, [])])
S_CT = (s_ct, [(6, [0]), (5, [3]), (0, []), (1, [2]), (3, []), (2, [1]), (4, [])])


def _set(m, k, v):
    m[k] = v
    return []


S_C = ([
    (0, lambda m: []),
    (3, lambda m: _set(m, 't', m[0] + m[3])),
    (1, lambda m: _set(m, 'u', m[0] - m[1]) + [(2, m[1] + m[3])]),
    (4, lambda m: _set(m, 't', m['t'] - m[4])),
    (2, lambda m: _set(m, 'u', m['u'] + m[2]) + [(1, m[2] + m[4])]),
    (6, lambda m: [(0, m['t'] + m[6])]),
    (5, lambda m: [(3, m['u'] + m[5])]),
], [0, 3, 4, 't', 'u'])
S_AT = ([
    (0, lambda m: []),
    (1, lambda m: _set(m, 'u', m[0] + m[1])),
    (5, lambda m: _set(m, 't', m[0] - m[5]) + [(2, m[1] + m[5])]),
    (4, lambda m: _set(m, 't', m['t'] + m[4])),
    (6, lambda m: _set(m, 'u', m['u'] - m[6]) + [(1, m[4] + m[6])]),
    (2, lambda m: [(0, m['t'] + m[2])]),
    (3, lambda m: [(3, m['u'] + m[3])]),
], [0, 1, 4, 't', 'u'])


class Vec:
    def __init__(self, x):
        self.x = list(x)

    def __add__(self, o):
        return Vec(a + b for a, b in zip(self.x, o.x))

    def __sub__(self, o):
        return Vec(a - b for a, b in zip(self.x, o.x))


def two_level_in(f, blk):
    f, order = f
    q = [None] * 4
    for o, needs in order:
        for k in needs:
            q[k] = Vec(blk(2 * (k // 2) + i, 2 * (k % 2) + j) for i in range(2) for j in range(2))
            yield None, None
        v = f(*q, only=o)
        x = [TIEF[0](v.x[k if f is s_a else k ^ SWAP[o]], k in TIE2) for k in range(4)]
        for i, _ in order:
            yield 7 * o + i, f(*x, only=i)


class Parked:
    def __init__(self, ref, base, rows, keep):
        self.ref, self.base, self.rows, self.keep, self.fresh = ref, base, rows, keep, {}

    def __getitem__(self, k):
        if k in self.fresh:
            return self.fresh[k]
        return self.ref[self.base + self.keep.index(k), pl.ds(0, self.rows), :]

    def __setitem__(self, k, v):
        self.ref[self.base + self.keep.index(k), pl.ds(0, self.rows), :] = v

    def arrive(self, k, v):
        self.fresh = {k: v}
        if k in self.keep:
            self[k] = v


EARLY = 2
N_SEM = 5

PACE = []
TIEF = [None]
TIE2, WT, WB, WA, LAG = [0], [5], [0], [0], [2]


def two_level_out(scheme, prod, emit, cost, park, rows):
    steps, keep = scheme
    ref, base = park
    outer = [Parked(ref, base + 5 * k, rows, keep) for k in range(4)]
    for o, after_o in steps:
        inner = {}
        for i, after_i in steps:
            for p in prod(7 * o + i):
                PACE.append(p)
                inner[i] = inner[i] + p if i in inner else p
                yield rows / 4
            for k, v in after_i(inner):
                if scheme is S_C:
                    k ^= SWAP[o]
                outer[k].arrive(o, v)
                for K, w in after_o(outer[k]):
                    emit(2 * (K // 2) + k // 2, 2 * (K % 2) + k % 2, w)
                    yield cost


def _table(text):
    return [tuple('-0+'.index(ch) - 1 for ch in row) for row in text.split()]


H_A = _table('+00-++000+-0 +0000000000+ 0++000-++00+ +00000000000 +0-000000000 0+0000000000 0+0000-++000 '
             '00000000000+ 000000+--000 000000000+0- 0000000000+0 000000+0-000 000000+00000 000+--0000+0 '
             '000+--000000 00000+000000 000+0-000000 0+000+-+0000 00000+-00000 0000++-000-0')
H_B = _table('+-0000 +0000+ 0000+- 0+000+ 00000+ 000+00 00+0-+ +000+0 00+000 +00000 00+000 00+0-0 +000+0 '
             '+-0-00 000+00 0+000+ 0+0+00 00+--+ 0+-++0 +-+-00')
H_C = _table('0000000- +000000+ +0000000 0+00000- --000000 0+000-00 +0000+00 -00000+0 +000-000 000000++ '
             '00+000+0 0000++00 00+0+000 00+0000- 000-000- 000+0+00 00++0000 00000-00 00+00-00 00+00000')
H_B_SET = list(dict.fromkeys(H_B))
SHORT = (3, 4, 6)
GU_A0 = [sum(14 if k in SHORT else 20 for k in range(o)) for o in range(7)]
GU_B0 = [sum(7 if k in SHORT else 16 for k in range(o)) for o in range(7)]
SWAP = (0, 1, 0, 0, 1, 1, 1)


def combo(row, x, memo):
    terms = [(k, c) for k, c in enumerate(row) if c]
    acc = x[terms[0][0]]
    for n in range(2, len(terms) + 1):
        key = tuple(terms[:n])
        if key not in memo:
            k, c = terms[n - 1]
            memo[key] = acc + x[k] if c > 0 else acc - x[k]
        acc = memo[key]
    return acc


class Ragged(dict):
    def __add__(self, o):
        return Ragged({k: self[k] + o[k] if k in self and k in o else (self.get(k) if k in self else o[k]) for k in {**self, **o}})

    def __sub__(self, o):
        return Ragged({k: self[k] - o[k] if k in o else self[k] for k in self})


def wide_in(side, blk, n_first, n_second):
    f, order = S_A if side == 'a' else S_B
    k0, nk = (0, n_first), (n_first, n_second)
    q = [None] * 4
    for o, needs in order:
        for k in needs:
            R, C = divmod(k, 2)
            if side == 'a':
                q[k] = Ragged({(i, l): blk(4 * R + i, k0[C] + l) for i in range(4) for l in range(nk[C])})
            else:
                q[k] = Ragged({(l, j): blk(k0[R] + l, 2 * C + j) for l in range(nk[R]) for j in range(2)})
            yield None, None, None
        v = f(*q, only=o)
        three = (n_second if o in SHORT else n_first) == 3
        if side == 'a' and three:
            x = [v[i, l] for i in range(4) for l in range(3)]
            memo = {}
            for r, row in enumerate(H_A):
                yield o, r, TIEF[0](combo(row, x, memo), r % WT[0] == 0)
        elif side == 'a':
            for i in range(2):
                x = [TIEF[0](v[i + 2 * p, l], 2 * p + l in WA) for p in range(2) for l in range(2)]
                for r, _ in order:
                    yield o, 7 * i + r, s_a(*x, only=r)
        else:
            x = [TIEF[0](v[l, j ^ SWAP[o]], 2 * l + j in WB) for l in range(3 if three else 2) for j in range(2)]
            memo = {}
            for r, row in enumerate(H_B_SET if three else order):
                yield (o, r, combo(row, x, memo)) if three else (o, row[0], s_b(*x, only=row[0]))


def wide_out(groups, prod, emit, park, rows):
    ref, base = park
    steps, keep = S_C
    outer = [Parked(ref, base + 6 * k, rows, keep + ['part']) for k in range(8)]

    def finish(o, after_o, k, v):
        k ^= SWAP[o]
        outer[k].arrive(o, v)
        for K, w in after_o(outer[k]):
            emit(4 * (K // 2) + k // 2, 2 * (K % 2) + k % 2, w)

    for o, after_o in steps:
        three, twos = groups(o)
        for i in range(2 if twos else 0):
            inner = {}
            for r, after_r in steps:
                for g in twos:
                    p = prod(g, o, 7 * i + r, r)
                    PACE.append(p)
                    inner[r] = inner[r] + p if r in inner else p
                    yield rows / 4
                for k, v in after_r(inner):
                    k = 2 * (i + 2 * (k // 2)) + k % 2
                    if three is None:
                        finish(o, after_o, k, v)
                    else:
                        outer[k]['part'] = v
        if three is not None:
            acc = {}
            for r, row in enumerate(H_C):
                p = prod(three, o, r, H_B_SET.index(H_B[r]))
                PACE.append(p)
                yield rows / 4
                for k, c in enumerate(row):
                    if c:
                        if k not in acc and twos:
                            acc[k] = (1, outer[k]['part'])
                        if k not in acc:
                            acc[k] = (c, p)
                        else:
                            sign, a = acc[k]
                            acc[k] = (sign, a + p) if sign == c else (1, a - p if sign > 0 else p - a)
                        if not any(later[k] for later in H_C[r + 1:]):
                            sign, a = acc.pop(k)
                            finish(o, after_o, k, a if sign > 0 else -a)


def interleave(*streams, tie2=(0,), wt=5, wb=(0,), lag=2):
    TIE2[:], WT[0], WB[:], LAG[0] = tie2, wt, wb, lag
    done = [0.0] * len(streams)
    live = list(range(len(streams)))
    while live:
        k = min(live, key=lambda n: done[n] / streams[n][1])
        try:
            done[k] += next(streams[k][0])
        except StopIteration:
            live.remove(k)


def chain(*streams):
    def gen():
        for g, _ in streams:
            yield from g
    return gen(), sum(c for _, c in streams)


def run(stream):
    interleave((stream[0], 1))


def dot(a, b):
    return jnp.dot(a, b, preferred_element_type=F32)


def dot_nt(a, b):
    return jax.lax.dot_general(a, b, (((1,), (1,)), ((), ())), preferred_element_type=F32)


def ld(ref, i, r0=0, rows=None):
    rows = ref.shape[1] if rows is None else rows
    return pltpu.bitcast(ref.bitcast(jnp.uint32)[i, pl.ds(r0 // 2, rows // 2), :], BF16)


def phi(t):
    return jnp.where(t > 0, t + 1.0, jnp.exp(t)) + 1e-6


def kernel(x_hbm, wqkv_hbm, wo_hbm, wg_hbm, wu_hbm, wd_hbm, c_hbm, wmod_hbm, o_hbm, c_v,
           x_v, wqkv_v, wo_v, wg_v, wu_v, wd_v, wmod_v, o_v,
           modc, xT, pqT, zacc, gacc, kA, qA, mA, guA, dA,
           hB, gA, pB, h2B, actT, aB, m_v, wT, pkT, park, rowv, sem, osem):
    tokens = lambda t: pl.ds(t * TM, TM)
    cols = lambda src, j, dst, c0=0, n=D: (src.at[:, pl.ds(j * D + c0, n)], dst.at[j, :, pl.ds(c0, n)])
    rows_of = lambda src, dst, r0, n: (src.at[pl.ds(r0, n)], dst.at[pl.ds(r0, n)])
    x_tile = lambda t: rows_of(x_hbm, x_v, t * TM, TM)
    gate_rows = lambda f0, f1: [rows_of(wg_hbm, wg_v, f0, f1 - f0), rows_of(wu_hbm, wu_v, f0, f1 - f0)]
    batches = [
        ('wk0', [(c_hbm, c_v), cols(wqkv_hbm, 1, wqkv_v, 0, 256)]),
        ('x0', [x_tile(0)]),
        ('ca', [cols(wmod_hbm, 1, wmod_v)]),
        ('wk1', [cols(wqkv_hbm, 1, wqkv_v, 256, 384)]),
        ('x1', [x_tile(1)]),
        ('wq', [cols(wqkv_hbm, 0, wqkv_v)]),
        ('sa', [cols(wmod_hbm, 0, wmod_v)]),
        ('x2', [x_tile(2)]),
        ('x3', [x_tile(3)]),
        ('gu01', gate_rows(0, 512)),
        ('gu23', gate_rows(512, 1024) + [cols(wqkv_hbm, 2, wqkv_v), (wo_hbm, wo_v)]),
        ('mod', [cols(wmod_hbm, j, wmod_v) for j in range(2, 5)]),
        ('gu456', gate_rows(1024, F)),
        ('wd', [(wd_hbm, wd_v), cols(wmod_hbm, 5, wmod_v)]),
    ] + [('fence%d' % k, [(c_hbm, c_v)]) for k in range(3)]
    fetch = {name: [pltpu.make_async_copy(a, b, sem.at[k % N_SEM]) for a, b in pairs]
             for k, (name, pairs) in enumerate(batches)}
    waiting, flying = list(fetch), []

    def request(last):
        while last in waiting:
            flying.append(waiting.pop(0))
            assert len(flying) <= N_SEM
            for cp in fetch[flying[-1]]:
                cp.start()

    def arrived(last):
        while last in flying:
            for cp in fetch[flying.pop(0)]:
                cp.wait()

    out_blocks = [(t, 0, D) for t in range(NT - 1)] + [(NT - 1, 8 * r0, 8 * sub) for r0, sub in D_PIECES]
    cp_o = {(t, e0): pltpu.make_async_copy(o_v.at[tokens(t), pl.ds(e0, n)], o_hbm.at[tokens(t), pl.ds(e0, n)], osem.at[k])
            for k, (t, e0, n) in enumerate(out_blocks)}

    def stream(cost):
        return lambda f: lambda *a: (f(*a), cost(*a) if callable(cost) else cost)

    strip = lambda n: pl.ds(16 * n, 16)
    TIEF[0] = lambda v, on: tie(v, on)
    park_turn = [0]
    PACE.clear()
    never = []

    def tie(v, on=True):
        if not (on and len(PACE) >= LAG[0]):
            return v
        p = PACE[-LAG[0]][0:8]
        return jnp.concatenate([jnp.where(never[0], p, v[r:r + 8]) for r in range(0, v.shape[0], 8)], axis=0)

    def next_park():
        park_turn[0] ^= 1
        return park, 48 * park_turn[0]

    def put_a(dst, base, blk, rows, r0=0):
        for n in range(r0 // 16, (r0 + rows) // 16):
            for r, v in two_level_in(S_A, lambda i, l: blk(i, l, n)):
                if r is not None:
                    dst[base + r, strip(n), :] = v.astype(BF16)
                yield 1 if r is not None else 2
            for i in range(4):
                dst[base + 49 + i, strip(n), :] = blk(i, 4, n).astype(BF16)
                yield 1

    def put_b(dst, base, blk):
        for n in range(L // 16):
            for r, v in two_level_in(S_B, lambda l, j: blk(l, j, n)):
                if r is not None:
                    dst[base + r, strip(n), :] = v.astype(BF16)
                yield 1 if r is not None else 4
            for j in range(4):
                dst[base + 49 + j, strip(n), :] = blk(4, j, n).astype(BF16)
                yield 2

    def mm640(a_ref, a0, b_ref, b0, split, emit):
        for r0, sub in split:
            def out(i, j, v):
                emit(i, j, r0, sub, v + dot(ld(a_ref, a0 + 49 + i, r0, sub), ld(b_ref, b0 + 49 + j)))
            yield from two_level_out(
                S_C, lambda r: [dot(ld(a_ref, a0 + r, r0, sub), ld(b_ref, b0 + r))], out, sub / 4, next_park(), sub)

    wT_blk = lambda split: lambda i, l, n: wT[l, pl.ds(feature(split, i, 16 * n), 16), :]

    @stream(lambda w, e0, e1: 100 * (e1 - e0))
    def turn_proj(w, e0, e1):
        for e in range(e0, e1):
            for l in range(5):
                wT[l, pl.ds(e * L, L), :] = wqkv_v[w, pl.ds(l * L, L), pl.ds(e * L, L)].astype(F32).T
                yield 20

    @stream(lambda dst, r0, rows: rows * 4)
    def prep_proj(dst, r0, rows):
        blk = lambda i, l, n: wT_blk(P_PIECES)(i, l, n) * rowv[1, :, pl.ds(l * L, L)]
        yield from put_a(dst, 0, blk, rows, r0)

    silu_c = []

    @stream(200)
    def mod_vec(j, plus_one):
        for l in range(5):
            row = dot(silu_c[0], wmod_v[j, :, pl.ds(l * L, L)])[0:1]
            if plus_one:
                row = row + 1.0
            modc[j, pl.ds(l * L, L), :] = jnp.broadcast_to(row, (L, L)).T
            yield 40

    @stream(100)
    def mod_row(j, plus_one):
        row = dot(silu_c[0], wmod_v[j])
        rowv[j] = row + 1.0 if plus_one else row
        yield 100

    @stream(200)
    def proj_bias(w):
        shift = rowv[0]
        hi = shift.astype(BF16).astype(F32)
        two = jnp.where(jax.lax.broadcasted_iota(jnp.int32, shift.shape, 0) == 0, hi, shift - hi).astype(BF16)
        for l in range(5):
            b = dot(two, wqkv_v[w, :, pl.ds(l * L, L)])
            modc[w, pl.ds(l * L, L), :] = jnp.broadcast_to(b[0:1] + b[1:2], (L, L)).T
            yield 40

    def fold(v):
        return jnp.sum(v.reshape(-1, 8, L), axis=0)

    stats = {}

    def ln_stats(t, sums):
        stats[t] = []
        for j in range(4):
            m = jnp.broadcast_to(jnp.sum(sums[j], axis=0, keepdims=True) * (1.0 / D), (8, L))
            acc = None
            for l in range(5):
                d = xT[4 * t + j, pl.ds(l * L, L), :].reshape(-1, 8, L) - tie(m)
                sq = jnp.sum(d * d, axis=0)
                acc = sq if acc is None else acc + sq
                yield 12
            v = jnp.sum(acc, axis=0, keepdims=True) * (1.0 / D)
            stats[t].append((m, jnp.broadcast_to(jax.lax.rsqrt(v + 1e-5), (16, L))))

    def norm_b(dst, t):
        def blk(l, j, n):
            r = pl.ds(l * L + 16 * n, 16)
            m, rstd = tie(stats[t][j][0]), stats[t][j][1]
            return (xT[4 * t + j, r, :] - jnp.concatenate([m, m], axis=0)) * rstd
        yield from put_b(dst, 0, blk)

    def load_x(t, sums):
        for j in range(4):
            for l in range(5):
                v = x_v[pl.ds(t * TM + j * L, L), pl.ds(l * L, L)].astype(F32).T
                xT[4 * t + j, pl.ds(l * L, L), :] = v
                sums[j] = fold(v) if l == 0 else sums[j] + fold(v)
                yield 20

    @stream(400 + 240)
    def load(t):
        sums = [None] * 4
        yield from load_x(t, sums)
        yield from ln_stats(t, sums)

    @stream(640)
    def comb(t):
        yield from norm_b(hB[t], t)

    @stream(lambda t, split=P_PIECES: 65 / 4 * sum(p[1] for p in split))
    def k_proj(t, split=P_PIECES):
        def emit(i, j, r0, rows, v):
            r = pl.ds(4 * r0 + i * rows, rows)
            pkT[4 * (t % 2) + j, r, :] = v if t < EARLY else phi(v + modc[1, r, :])
        yield from mm640(kA, 0, hB[t], 0, split, emit)

    @stream(65 * 40)
    def q_proj(t):
        def emit(i, j, r0, rows, v):
            r = pl.ds(4 * r0 + i * rows, rows)
            pqT[4 * t + j, r, :] = v if t < 1 else phi(v + modc[0, r, :])
        yield from mm640(qA, 0, hB[t], 0, P_PIECES, emit)

    @stream(lambda t, strips=range(RB // 16): len(strips) * (101 if t < EARLY else 69))
    def g_pre(t, strips=range(RB // 16)):
        for n in strips:
            pk = {}
            def blk(i, j):
                r = pl.ds(feature(G_PIECES, i, 16 * n), 16)
                v = pkT[4 * (t % 2) + j, r, :]
                pk[i, j] = phi(v + tie(modc[1, r, :])) if t < EARLY else v
                gA[t][49 + 4 * i + j, strip(n), :] = pk[i, j].astype(BF16)
                return pk[i, j]
            for r, v in two_level_in(S_CT, blk):
                if r is not None:
                    gA[t][r, strip(n), :] = v.astype(BF16)
                yield 1 if r is not None else 12 if t < EARLY else 4
            for i in range(4):
                zs = (pk[i, 0] + pk[i, 1]) + (pk[i, 2] + pk[i, 3])
                r = pl.ds(feature(G_PIECES, i, 16 * n), 16)
                zacc[r, :] = zs if t == 0 else zacc[r, :] + zs
                yield 1

    @stream(lambda t0, split=G_PIECES: 65 / 2 * sum(p[1] for p in split))
    def g_acc(t0, split=G_PIECES):
        for r0, sub in split:
            prod = lambda ra, rb: (dot_nt(ld(gA[t], ra, r0, sub), ld(hB[t], rb)) for t in (t0, t0 + 1))
            def emit(i, l, v):
                r = pl.ds(4 * r0 + i * sub, sub)
                gacc[l, r, :] = v if t0 == 0 else gacc[l, r, :] + v
            yield from two_level_out(S_AT, lambda r: prod(r, r), emit, 0, next_park(), sub)
            for i in range(4):
                e = None
                for j in range(4):
                    for p in prod(49 + 4 * i + j, 49 + j):
                        PACE.append(p)
                        e = p if e is None else e + p
                        yield sub / 4
                emit(i, 4, e)

    @stream(lambda q: GU_CHUNKS[q][1] / 32 * 130)
    def prep_gu(q):
        f0, rows = GU_CHUNKS[q][0], GU_CHUNKS[q][1] // 2
        for n in range(rows // 16):
            def blk(i, l):
                w = wg_v if i < 4 else wu_v
                return w[pl.ds(f0 + (i % 4) * rows + 16 * n, 16), pl.ds(l * L, L)].astype(F32)
            for o, r, v in wide_in('a', blk, 3, 2):
                if o is not None:
                    guA[q][GU_A0[o] + r, strip(n), :] = v.astype(BF16)
                yield 1 if o is not None else 2

    @stream(lambda s: 200 * D_GROUPS[s][1])
    def turn_d(s):
        l0, nk = D_GROUPS[s]
        buf, b0 = (wT, 0) if s == 0 else (pkT, 4 * s - 4)
        for l in range(2 * nk):
            f0 = (l0 + l) * L
            for e in range(5):
                if f0 + L <= F:
                    w = wd_v[pl.ds(f0, L), pl.ds(e * L, L)].astype(F32)
                else:
                    w = jnp.concatenate([wd_v[pl.ds(f0, F - f0), pl.ds(e * L, L)].astype(F32),
                                         jnp.zeros((f0 + L - F, L), F32)], axis=0)
                buf[b0 + l, pl.ds(e * L, L), :] = w.T * modc[5, pl.ds(e * L, L), :]
                yield 20

    @stream(lambda s: 5 * (148 if s == 0 else 106))
    def prep_d(s):
        l0, nk = D_GROUPS[s]
        buf, b0 = (wT, 0) if s == 0 else (pkT, 4 * s - 4)
        for n in range(D // 8 // 16):
            blk = lambda i, l: buf[b0 + l, pl.ds(feature(D_PIECES, i, 16 * n, 8), 16), :]
            for o, r, v in wide_in('a', blk, nk, nk):
                if o is not None:
                    dA[s][(20 if s == 0 else 14) * o + r, strip(n), :] = v.astype(BF16)
                yield 1 if o is not None else 2

    @stream(2000)
    def mid():
        for j, (lo, hi) in enumerate(HEAD_ROWS):
            r = pl.ds(lo, hi - lo)
            g = jnp.concatenate([gacc[l, r, :] * rowv[1, 0:1, pl.ds(l * L, L)] + zacc[r, :] * rowv[0, 0:1, pl.ds(l * L, L)]
                                 for l in range(5)], axis=1).astype(BF16)
            kv = dot(g, wqkv_v[2, :, pl.ds(j * L, L)])
            yield 200
            rh = jax.lax.broadcasted_iota(jnp.int32, kv.shape, 0) + lo
            ch = jax.lax.broadcasted_iota(jnp.int32, kv.shape, 1) + j * L
            head = lambda v: (v * 3277) >> 16
            kv = jnp.where(head(rh) == head(ch), kv, 0.0).astype(BF16)
            mj = dot(kv, wo_v[pl.ds(j * L, L), :])
            plo = HEAD_ROWS[j - 1][1] if j else lo
            if plo > lo:
                m_v[pl.ds(lo, plo - lo), :] += mj[:plo - lo]
            m_v[pl.ds(plo, hi - plo), :] = mj[plo - lo:]
            yield 200

    @stream(25 * 20 + 600)
    def prep_m():
        for l in range(5):
            for e in range(5):
                wT[l, pl.ds(e * L, L), :] = m_v[pl.ds(l * L, L), pl.ds(e * L, L)].T * modc[2, pl.ds(e * L, L), :]
                yield 20
        yield from put_a(mA, 0, wT_blk(P_PIECES), RB)

    @stream(100)
    def z_final():
        for l in range(5):
            r = pl.ds(l * L, L)
            zacc[r, :] = jnp.broadcast_to(jnp.sum(zacc[r, :], axis=1, keepdims=True), (L, L))
            yield 20

    @stream(lambda t: 16 * (73 if t < 1 else 41) + 580)
    def attn_pre(t):
        row = jax.lax.broadcasted_iota(jnp.int32, (8, L), 0)
        low, bit2, bit1 = row < 4, (row & 2) == 0, (row & 1) == 0
        part, rden = {}, {}

        def weigh(g):
            r = pl.ds(40 * g, 40)
            z = zacc[r, :]
            part[g] = []
            for j in range(4):
                pq = pqT[4 * t + j, r, :]
                if t < 1:
                    pq = pqT[4 * t + j, r, :] = phi(pq + tie(modc[0, r, :]))
                w = pq * z
                a = w[0:8] + tie(w[8:16])
                b = w[24:32] + w[32:40]
                part[g].append(jnp.where(low, a, b) + pltpu.roll(jnp.where(low, b, a), 4, 0) + w[16:24])
                yield 12 if t < 1 else 4

        def fold2(m, d, a, b):
            return jnp.where(m, a, b) + jnp.where(m, pltpu.roll(a, 8 - d, 0), pltpu.roll(b, d, 0))

        def invert(g):
            p = part.pop(g)
            den = fold2(bit1, 1, fold2(bit2, 2, tie(p[0]), p[2]), fold2(bit2, 2, tie(p[1]), p[3]))
            rden[g] = 1.0 / (den + 1e-6)
            yield 5

        def scale(g):
            r = pl.ds(40 * g, 40)
            for j in range(4):
                q = tie(rden[g])
                ra = jnp.broadcast_to(q[j:j + 1], (8, L))
                rb = jnp.broadcast_to(q[4 + j:5 + j], (8, L))
                pqT[4 * t + j, r, :] *= jnp.concatenate([ra, ra, jnp.where(low, ra, rb), rb, rb], axis=0)
                yield 5

        n = D // 40
        for g in range(n + 2):
            if g < n:
                yield from weigh(g)
            if 0 <= g - 1 < n:
                yield from invert(g - 1)
            if 0 <= g - 2:
                yield from scale(g - 2)
        yield from put_b(pB[t % 2], 0, lambda l, j, n: pqT[4 * t + j, pl.ds(l * L + 16 * n, 16), :])

    sums2 = {}

    @stream(65 * 40)
    def attn(t):
        sums = sums2[t] = [None] * 4
        def emit(i, j, r0, rows, v):
            r = pl.ds(4 * r0 + i * rows, rows)
            x1 = xT[4 * t + j, r, :] + v
            xT[4 * t + j, r, :] = x1
            sums[j] = fold(x1) if sums[j] is None else sums[j] + fold(x1)
        yield from mm640(mA, 0, pB[t % 2], 0, P_PIECES, emit)

    @stream(240 + 8 * 110)
    def ffn_pre(t):
        yield from ln_stats(t, sums2[t])
        for n in range(L // 16):
            tied = {}
            def blk(l, j):
                r = pl.ds(l * L + 16 * n, 16)
                m, rstd = stats[t][j]
                if (l, j) not in tied:
                    for k in (range(3) if l < 3 else range(3, 5)):
                        tied[k, j] = tie(m) if k == l else tied[l, j]
                m = tied[l, j]
                return (xT[4 * t + j, r, :] - jnp.concatenate([m, m], axis=0)) * rstd * modc[4, r, :] + modc[3, r, :]
            for o, r, v in wide_in('b', blk, 3, 2):
                if o is not None:
                    h2B[t % 2][GU_B0[o] + r, strip(n), :] = v.astype(BF16)
                yield 1 if o is not None else 6

    @stream(lambda t, q, most=64: GU_CHUNKS[q][1] * 122 / 8)
    def gate_up(t, q, most=64):
        f0, rows = GU_CHUNKS[q][0], GU_CHUNKS[q][1] // 2
        for r0, sub in pieces(rows, most):
            held = {}
            def emit(i, j, v):
                held[i, j] = v
                if (i ^ 4, j) in held:
                    hg = 0.5 * held.pop((i & 3, j))
                    up = held.pop((4 + (i & 3), j))
                    actT[j, pl.ds(f0 + (i & 3) * rows + r0, sub), :] = (hg * up) * (1.0 + jnp.tanh(hg))
            prod = lambda g, o, ra, rb: dot(ld(guA[q], GU_A0[o] + ra, r0, sub), ld(h2B[t % 2], GU_B0[o] + rb))
            yield from wide_out(lambda o: (None, [0]) if o in SHORT else (0, []), prod, emit, next_park(), sub)

    @stream(lambda t, s: 8 * (116 if s == 0 else 53))
    def act_b(t, s):
        l0, nk = D_GROUPS[s]
        for n in range(L // 16):
            blk = lambda l, j: actT[j, pl.ds((l0 + l) * L + 16 * n, 16), :]
            for o, r, v in wide_in('b', blk, nk, nk):
                if o is not None:
                    aB[t % 2][s][(16 if s == 0 else 7) * o + r, strip(n), :] = v.astype(BF16)
                yield 1

    @stream(lambda t, split=D_PIECES: 7 * 48 / 4 * sum(p[1] for p in split))
    def down(t, split=D_PIECES):
        for r0, sub in split:
            def emit(i, j, v):
                xT[4 * t + j, pl.ds(8 * r0 + i * sub, sub), :] += v
            prod = lambda s, o, ra, rb: dot(ld(dA[s], (20 if s == 0 else 14) * o + ra, r0, sub),
                                            ld(aB[t % 2][s], (16 if s == 0 else 7) * o + rb))
            yield from wide_out(lambda o: (0, [1, 2]), prod, emit, next_park(), sub)

    @stream(lambda t, e0=0, n=D: n * 400 / D)
    def put_out(t, e0=0, n=D):
        for j in range(4):
            for l in range(e0 // L, (e0 + n) // L):
                o_v[pl.ds(t * TM + j * L, L), pl.ds(l * L, L)] = xT[4 * t + j, pl.ds(l * L, L), :].T.astype(BF16)
                yield 20
        cp_o[t, e0].start()


    request('x1')
    actT[:, pl.ds(F, 64), :] = jnp.zeros((4, 64, L), F32)

    def touch(i, carry):
        for ref in (modc, xT, pqT, gacc, kA, qA, mA, *guA, *dA, *hB, *gA, *pB, *h2B, actT, *aB[0], *aB[1], wT, pkT, park):
            ref[i, pl.ds(0, 16), :] = jnp.zeros((16, L), ref.dtype)
        zacc[pl.ds(pl.multiple_of(i * 8, 8), 8), :] = jnp.zeros((8, L), F32)
        m_v[pl.ds(pl.multiple_of(i * 8, 8), 8), pl.ds(0, L)] = jnp.zeros((8, L), F32)
        return carry
    jax.lax.fori_loop(0, 2, touch, 0)
    arrived('wk0')
    cf = c_v[...].astype(F32)
    silu_c.append(jnp.broadcast_to(cf * (1.0 / (1.0 + jnp.exp(-cf))), (16, D)).astype(BF16))
    never.append(jnp.broadcast_to(cf[:, :L], (8, L)) != jnp.broadcast_to(cf[:, :L], (8, L)))
    GU = lambda t, *qs, most=64: chain(*[gate_up(t, q, most) for q in qs])
    both = [0, 3]
    run(turn_proj(1, 0, 2))
    arrived('x0')
    run(chain(load(0), comb(0)))
    arrived('ca')
    request('wq')
    run(chain(mod_row(1, True), prep_proj(kA, 0, 64)))
    arrived('wk1')
    interleave(k_proj(0, P_PIECES[:1]), chain(turn_proj(1, 2, 5), prep_proj(kA, 64, 96)))
    arrived('x1')
    request('x2')
    interleave(k_proj(0, P_PIECES[1:]), chain(load(1), comb(1)))
    arrived('wq')
    request('x3')
    interleave(k_proj(1), chain(turn_proj(0, 0, 5), prep_proj(qA, 0, RB)))
    arrived('sa')
    request('gu01')
    interleave(q_proj(0), chain(mod_row(0, False), proj_bias(1), proj_bias(0), g_pre(0)), lag=4)
    arrived('x3')
    request('gu23')
    interleave(q_proj(1), chain(load(2), comb(2)), lag=4)
    interleave(k_proj(2), chain(g_pre(1, range(5)), load(3)))
    interleave(g_acc(0, G_PIECES[:1]), chain(g_pre(1, range(5, 10)), comb(3)), lag=4)
    interleave(k_proj(3), g_pre(2), lag=4)
    arrived('gu23')
    request('gu456')
    interleave(g_acc(0, G_PIECES[1:]), chain(g_pre(3), z_final(), prep_gu(0)), wt=3)
    interleave(g_acc(2), chain(attn_pre(0), prep_gu(1), prep_gu(2)), tie2=both)
    interleave(q_proj(3), mid(), attn_pre(1), tie2=both)
    arrived('gu456')
    request('wd')
    interleave(q_proj(2), chain(mod_vec(2, False), prep_m()))
    interleave(attn(0), chain(prep_gu(3), mod_vec(3, False), mod_vec(4, True)), wt=3)
    interleave(attn(1), ffn_pre(0), wb=[0, 2])
    interleave(GU(0, 0, 1, 2, most=32), chain(prep_gu(4), prep_gu(5)), wt=3)
    interleave(GU(0, 3, 4, most=32), chain(prep_gu(6), act_b(0, 0)), wt=3)
    interleave(GU(0, 5, 6), ffn_pre(1), wb=[0, 2])
    arrived('wd')
    request('fence0')
    interleave(chain(GU(1, 0, 1, 2, 3, 4, 5, 6), attn(2)),
               chain(mod_vec(5, False), act_b(0, 1), act_b(0, 2), turn_d(1), turn_d(2), turn_d(0), attn_pre(2),
                     prep_d(1), prep_d(2), prep_d(0)), tie2=both)
    arrived('fence0')
    request('fence1')
    interleave(down(0), chain(ffn_pre(2), act_b(1, 0), act_b(1, 1), act_b(1, 2)))
    interleave(GU(2, 0, 1, 2, 3), chain(put_out(0), attn_pre(3)), tie2=both)
    interleave(chain(GU(2, 4, 5, 6), attn(3)), act_b(2, 0), wb=[0, 2])
    arrived('fence1')
    request('fence2')
    interleave(down(1), ffn_pre(3))
    interleave(GU(3, 0, 1, 2), chain(act_b(2, 1), act_b(2, 2), put_out(1)))
    run(GU(3, 3, 4, 5, 6))
    arrived('fence2')
    interleave(down(2), chain(act_b(3, 0), act_b(3, 1), act_b(3, 2)))
    landed = list(cp_o.values())
    landed.pop(0).wait()
    interleave(down(3, D_PIECES[:1]), put_out(2))
    for p, (r0, sub) in enumerate(D_PIECES):
        landed.pop(0).wait()
        interleave(put_out(3, 8 * r0, 8 * sub), *([down(3, D_PIECES[p + 1:p + 2])] if p + 1 < len(D_PIECES) else []))
    for cp in landed:
        cp.wait()


@jax.jit
def pallas_adaLN_cond__linear_attn_block__swiglu_ffn__prompt_kernel(
        A_x, A_wqkv, A_wo, B_x, B_w_gate, B_w_up, B_w_down, c, w_mod):
    del B_x
    hbm = pl.BlockSpec(memory_space=pl.ANY)
    vm = pltpu.VMEM
    out = pl.pallas_call(
        kernel,
        out_shape=jax.ShapeDtypeStruct((S, D), BF16),
        in_specs=[hbm] * 6 + [hbm, hbm],
        out_specs=hbm,
        scratch_shapes=[
            vm((1, D), BF16), vm((S, D), BF16), vm((3, D, D), BF16), vm((D, D), BF16),
            vm((F, D), BF16), vm((F, D), BF16), vm((F, D), BF16), vm((6, D, D), BF16), vm((S, D), BF16),
            vm((6, D, L), F32),
            vm((S // L, D, L), F32),
            vm((S // L, D, L), F32),
            vm((D, L), F32),
            vm((5, D, L), F32),
            vm((53, RB, L), BF16), vm((53, RB, L), BF16), vm((53, RB, L), BF16),
            [vm((122, rows // 2, L), BF16) for _, rows in GU_CHUNKS],
            [vm((n, D // 8, L), BF16) for n in (140, 98, 98)],
            [vm((53, L, L), BF16)] * NT,
            [vm((65, RB, L), BF16)] * NT,
            [vm((53, L, L), BF16)] * 2,
            [vm((85, L, L), BF16)] * 2,
            vm((4, F + 64, L), F32),
            [[vm((n, L, L), BF16) for n in (112, 49, 49)]] * 2,
            vm((D, D), F32),
            vm((6, D, L), F32), vm((8, D, L), F32), vm((96, 80, L), F32),
            vm((2, 16, D), F32),
            pltpu.SemaphoreType.DMA((N_SEM,)), pltpu.SemaphoreType.DMA((NT - 1 + len(D_PIECES),)),
        ],
        compiler_params=pltpu.CompilerParams(
            vmem_limit_bytes=120 * 2**20, flags={'XLA_TPU_EVENLY_DISTRIBUTE_CRITICAL_NODES': True}),
    )(A_x.reshape(S, D), A_wqkv, A_wo, B_w_gate.T, B_w_up.T, B_w_down, c, w_mod)
    return out.reshape(1, S, D)
```
